```python
import os as _os
_os.environ.setdefault("JAX_PLATFORMS", "cpu")
import jax
import jax.numpy as jnp

def _softmax(x, axis=-1):
    return jax.nn.softmax(x, axis=axis)
def _gelu(x):
    return jax.nn.gelu(x, approximate=True)
def _silu(x):
    return jax.nn.silu(x)
def _sigmoid(x):
    return jax.nn.sigmoid(x)
def _layernorm(x, axis=-1, eps=1e-5):
    m = jnp.mean(x, axis=axis, keepdims=True)
    v = jnp.var(x, axis=axis, keepdims=True)
    return (x - m) / jnp.sqrt(v + eps)
def _scatter_add(tgt, idx, src, axis=0):
    return tgt.at[idx].add(src)
def _segment_sum(src, seg, n):
    return jax.ops.segment_sum(src, seg, n)
class _Rng:
    def __init__(self, key):
        self._k = key
    def _next(self):
        self._k, sub = jax.random.split(self._k)
        return sub
    def normal(self, shape):
        return jax.random.normal(self._next(), shape, dtype=jnp.bfloat16)
    def randint(self, lo, hi, shape):
        return jax.random.randint(self._next(), shape, lo, hi, dtype=jnp.int32)
    def uniform(self, shape, lo=0.0, hi=1.0):
        return jax.random.uniform(self._next(), shape, jnp.bfloat16, lo, hi)
    def permutation(self, n):
        return jax.random.permutation(self._next(), n)


kernel_name = 'standalone__mixer_token_mlp__sampling'

def setup_inputs():
    _rng = _Rng(jax.random.key(int.from_bytes(__import__("os").urandom(4), "little")))
    _w = (lambda a: (lambda t: t.astype(jnp.bfloat16) if jnp.issubdtype(t.dtype, jnp.floating) else t)(jnp.asarray(a)))
    B, S, D, F = 32, 16, 1024, 3584
    return {
        "x": _w((lambda *s: _rng.normal(s) * 0.05)(B, S, D)),
        "w1": _w((lambda *s: _rng.normal(s) * 0.05)(S, F) * (S ** -0.5)),
        "b1": _w((lambda *s: _rng.normal(s) * 0.05)(F) * 0.02),
        "w2": _w((lambda *s: _rng.normal(s) * 0.05)(F, S) * (F ** -0.5)),
        "b2": _w((lambda *s: _rng.normal(s) * 0.05)(S) * 0.02),
    }

def reference(x, w1, b1, w2, b2):
    B, S, D = x.shape
    h = _layernorm(x, axis=-1)
    u = jnp.einsum("bsd,sf->bdf", h, w1) + b1
    u = _gelu(u)
    y = jnp.einsum("bdf,fs->bds", u, w2) + b2
    return (lambda x, *d: x.transpose(*d))(y, 0, 2, 1)
```

```python
import functools
import numpy as np
import jax
import jax.numpy as jnp
from jax import lax
import jax.experimental.pallas as pl
import jax.experimental.pallas.tpu as pltpu

CFG = dict(NB=2, PAT="p1", LAG=17, VPOS=0, OFF=11, LIN=1, LP=0, CW=2, KS=2, LB=16, EP=2, CL="c0123", AJ=0, RAW=3, LNPOS=3, LASTV=1)

_C1 = float(np.sqrt(2.0 / np.pi))
_C2 = _C1 * 0.044715
_A = float(np.cbrt(_C2))
_CZ = _C1 / _A
TD = 512
NJ = TD // 128
f32, bf16 = jnp.float32, jnp.bfloat16


def _mm(a, b):
    return lax.dot_general(a, b, (((1,), (0,)), ((), ())), preferred_element_type=f32)


def _plan(n_tiles, PAT, VPOS, LASTV):
    pat = [int(c) for c in str(PAT).lstrip("p")]
    tiles = []
    for c in range(n_tiles):
        nv = pat[c % len(pat)] if c < n_tiles - 1 else LASTV
        order = list(range(15, -1, -1))
        if VPOS == 0:
            v, m = order[16 - nv:], order[:16 - nv]
        else:
            v, m = order[:nv], order[nv:]
        tiles.append((m, v))
    return tiles


def _kernel(x_hbm, w1_ref, b1_ref, w2t_ref, b2_ref, o_hbm,
            x_ref, o_ref, lhs_ref, wv_ref, hf_ref, cu_ref, sems, idx_ref, *, NB, PAT, LAG, VPOS, OFF, LIN, LP, CW, KS, LB, EP, CL, AJ, RAW, LNPOS, LASTV):
    B, S, D = x_ref.shape
    F = w1_ref.shape[1]
    NT = F // 128
    KA = S + 8
    tiles = _plan(NT, PAT, VPOS, LASTV)
    cl, cw, ch, cs = [slice(8 * int(c), 8 * int(c) + 8) for c in CL[1:]]
    ch = slice(16 * ch.start, 16 * ch.start + 128)
    cp0 = pltpu.make_async_copy(x_hbm.at[pl.ds(0, NB)], x_ref.at[pl.ds(0, NB)], sems.at[0])
    cp1 = pltpu.make_async_copy(x_hbm.at[pl.ds(NB, B - NB)], x_ref.at[pl.ds(NB, B - NB)], sems.at[1])
    cp0.start()
    cp1.start()

    w1 = w1_ref[...].astype(f32)
    b1 = b1_ref[...].astype(f32)
    w2t = w2t_ref[...].astype(f32)
    row = lax.broadcasted_iota(jnp.int32, (8, 128), 0)
    vidx, was = {}, []
    nm = 0
    for c in range(NT):
        wa = jnp.concatenate([w1[:, c * 128:(c + 1) * 128], jnp.where(row < 2, b1[c:c + 1], 0.0)], axis=0)
        was.append(wa)
        wt = jnp.concatenate([wa, jnp.zeros((128 - KA, 128), f32)], axis=0).T
        m, v = tiles[c]
        for r in m:
            lhs_ref[nm, cl, :] = wt[8 * r:8 * r + 8]
            nm += 1
        for r in v:
            j = len(vidx)
            vidx[c, r] = j
            for k in range(S + 1):
                col = jnp.broadcast_to(wt[8 * r:8 * r + 8, k:k + 1], (8, 128))
                wv_ref[j * (S + 1) + k, cw, :] = col * _A if k == S else col
    for c in range(NT):
        for z in range(2):
            lhs_ref[nm + 2 * c + z, cl, :] = w2t[8 * z:8 * z + 8, c * 128:(c + 1) * 128]
    wa = jnp.concatenate(was, axis=1)
    ml = lax.dot_general(w2t, wa, (((1,), (1,)), ((), ())), preferred_element_type=f32)
    m_hi = ml[:, :S].astype(bf16).astype(f32)
    m_hl = jnp.concatenate([m_hi, ml[:, :S] - m_hi], axis=1)
    rr = lax.broadcasted_iota(jnp.int32, (S, S), 0)
    cc = lax.broadcasted_iota(jnp.int32, (S, S), 1)
    b2c = jnp.sum(jnp.where(rr == cc, b2_ref[...].astype(f32), 0.0), axis=1, keepdims=True)
    bias = jnp.broadcast_to(b2c + (0.5 * ml[:, S:S + 1] if LIN else 0.0), (S, 128))

    a_hi = float(np.float32(_A).astype(bf16).astype(np.float32))
    a_lo = _A - a_hi
    ones = jnp.where(row == 0, a_hi, jnp.where(row == 1, a_lo, 0.0))
    HPB = 2 * D // 128

    def layernorm(b, bx):
        x = x_ref[bx].astype(f32)
        mu = jnp.mean(x, axis=-1, keepdims=True)
        xc = x - mu
        var = jnp.mean(xc * xc, axis=-1, keepdims=True)
        h = xc * (lax.rsqrt(var + 1e-5) * _A)
        for jj in range(D // 128):
            hf_ref[b, jj, :, ch] = h[:, 128 * jj:128 * jj + 128]

    idx_ref[0] = 0
    cp0.wait()
    for bb in range(NB):
        layernorm(bb, bb)
    for z in range(cu_ref.shape[0]):
        cu_ref[z, cs, :] = jnp.zeros((8, 128), f32)
    cp1.wait()

    def act(v):
        t = jnp.tanh(v * (v * v + _CZ))
        return v * t if LIN else v * t + v

    def make_vstep(hsel):
        part, done = {}, {}

        def vstep(q, c, r, j0, k0):
            b, jb = hsel(q)
            j = vidx[c, r] * (S + 1)
            ws = [wv_ref[j + k, cw, :] for k in range(k0, k0 + KS)]
            wb = wv_ref[j + S, cw, :] if k0 == 0 else None
            for jj in range(j0, j0 + CW):
                ts = [w * hf_ref[b, jb + jj, k:k + 1, ch] for w, k in zip(ws, range(k0, k0 + KS))]
                while len(ts) > 1:
                    ts = [ts[z] + ts[z + 1] for z in range(0, len(ts), 2)]
                v = (wb if k0 == 0 else part[q, c, r, jj]) + ts[0]
                part[q, c, r, jj] = v
                if k0 + KS == S:
                    done[q, c, r, jj] = act(v)
        return vstep, done

    def vsteps(q, c):
        return [(q, c, r, j0, k0) for r in tiles[c][1] for j0 in range(0, NJ, CW) for k0 in range(0, S, KS)]

    def mm2(c, g):
        return _mm(jnp.concatenate([lhs_ref[nm + 2 * c + z, cl, :] for z in range(2)], axis=0), jnp.concatenate(g, axis=0))

    def emit(slot, jb, a):
        y = a * (0.5 / _A) + jnp.tile(bias, (1, NJ))
        o_ref[slot, :, 128 * jb:128 * jb + TD] = y.astype(o_ref.dtype)

    lastm = tiles[NT - 1][0]

    def finish_deferred(slot, done, q):
        g = {}
        for z, r in enumerate(lastm):
            u = jnp.concatenate([cu_ref[NJ * z + jj, cs, :] for jj in range(NJ)], axis=1)
            g[r] = act(u) if z >= len(lastm) - RAW else u
        for r in tiles[NT - 1][1]:
            g[r] = jnp.concatenate([done.pop((q, NT - 1, r, jj)) for jj in range(NJ)], axis=1)
        a = jnp.concatenate([jnp.concatenate([cu_ref[NJ * (len(lastm) + z) + jj, cs, :] for jj in range(NJ)], axis=1)
                             for z in range(2)], axis=0)
        emit(slot, D // 128 - NJ, a + mm2(NT - 1, [g[r] for r in range(16)]))

    def out_copy(grp):
        return pltpu.make_async_copy(o_ref.at[pl.ds(grp * NB + 1, NB)], o_hbm.at[pl.ds(grp * NB, NB)], sems.at[2])

    def body(it, carry):
        cgs = [(bb, j0) for bb in range(NB) for j0 in range(0, D // 128, NJ)]
        flat = [(q, c, r) for q in range(len(cgs)) for c in range(NT) for r in tiles[c][0]]
        per = len(flat) // len(cgs)
        ends, n = [(-1, NT - 1, 0)], 0
        for q in range(len(cgs)):
            for c in range(NT):
                n += len(tiles[c][0])
                ends.append((q, c, n))
        ends.pop()
        gs, acc, us = {}, {}, {}
        pos = 0
        steps = [st for (q, c, n) in ends[1:] for st in vsteps(q, c)]
        anchored = {}
        if steps:
            endof = {(q, c): n for (q, c, n) in ends}
            base = [m * ends[-1][2] // len(steps) for m in range(len(steps))]
            shift = min(endof[st[:2]] + OFF - b_ for st, b_ in zip(steps, base))
            for st, b_ in zip(steps, base):
                anchored.setdefault(max((b_ + shift) // EP * EP, 0), []).append(st)
        dummy = idx_ref[0]
        prev = jnp.maximum(it * NB - 1, 0)
        vstep, done = make_vstep(lambda q: (prev, D // 128 - NJ) if q < 0 else (it * NB + cgs[q][0], cgs[q][1]))
        for st in vsteps(-1, NT - 1):
            vstep(*st)

        for i, (q, c, n) in enumerate(ends):
            tgt = min(n + LAG, len(flat))
            while pos < tgt:
                q1 = flat[pos][0]
                stop = min(tgt, (q1 + 1) * per)
                bb, jb = cgs[q1]
                h = jnp.concatenate([hf_ref[it * NB + bb, jb + jj, :, ch] for jj in range(NJ)], axis=1)
                if LIN and pos == q1 * per:
                    acc[q1] = _mm(m_hl, jnp.concatenate([h, h], axis=0))
                lhs = [lhs_ref[t - q1 * per, cl, :KA] for t in range(pos, stop)]
                u = _mm(jnp.concatenate(lhs, axis=0), jnp.concatenate([h, jnp.tile(ones, (1, NJ))], axis=0))
                for t in range(stop - pos):
                    us[pos + t] = u[8 * t:8 * t + 8]
                    if pos + t < len(flat) - RAW:
                        gs[flat[pos + t]] = act(u[8 * t:8 * t + 8])
                for t in range(pos, stop):
                    if t in anchored:
                        if LB and t - LB >= 0:
                            wv_ref[dummy, cs, :] = us[t - LB][:, 128 * AJ:128 * AJ + 128]
                        for st in anchored.pop(t):
                            vstep(*st)
                pos = stop
            if pos == len(flat):
                for t in sorted(anchored):
                    for st in anchored.pop(t):
                        vstep(*st)
            if q < 0:
                finish_deferred(it * NB, done, q)
                continue
            for r in tiles[c][1]:
                gs[q, c, r] = jnp.concatenate([done.pop((q, c, r, jj)) for jj in range(NJ)], axis=1)
            p = mm2(c, [gs.pop((q, c, r)) for r in range(16)])
            acc[q] = acc[q] + p if q in acc else p
            if c == NT - 1:
                emit(it * NB + cgs[q][0] + 1, cgs[q][1], acc.pop(q))
            if c == LNPOS and cgs[q][1] == 0:
                b = (it + 1) * NB + cgs[q][0]
                layernorm(b, jnp.minimum(b, B - 1))
        ql = len(cgs) - 1
        for z, r in enumerate(lastm):
            u = gs.pop((ql, NT - 1, r)) if z < len(lastm) - RAW else us[len(flat) - len(lastm) + z]
            for jj in range(NJ):
                cu_ref[NJ * z + jj, cs, :] = u[:, 128 * jj:128 * jj + 128]
        for z in range(2):
            for jj in range(NJ):
                cu_ref[NJ * (len(lastm) + z) + jj, cs, :] = acc[ql][8 * z:8 * z + 8, 128 * jj:128 * jj + 128]

        @pl.when(it > 0)
        def _():
            out_copy(it - 1).start()
        return carry

    lax.fori_loop(0, B // NB, body, 0)
    vstep, done = make_vstep(lambda q: (B - 1, D // 128 - NJ))
    for st in vsteps(-1, NT - 1):
        vstep(*st)
    finish_deferred(B, done, -1)
    out_copy(B // NB - 1).start()
    pltpu.make_async_copy(o_ref.at[pl.ds(1, B)], o_hbm, sems.at[2]).wait()


@jax.jit
def pallas_standalone__mixer_token_mlp__sampling_kernel(x, w1, b1, w2, b2):
    B, S, D = x.shape
    F = w1.shape[1]
    tiles = _plan(F // 128, CFG["PAT"], CFG["VPOS"], CFG["LASTV"])
    nm = sum(len(m) for m, _ in tiles)
    nv = sum(len(v) for _, v in tiles)
    kern = functools.partial(_kernel, **CFG)
    vmem = pl.BlockSpec(memory_space=pltpu.VMEM)
    return pl.pallas_call(
        kern,
        in_specs=[pl.BlockSpec(memory_space=pl.ANY), vmem, vmem, vmem, vmem],
        out_specs=pl.BlockSpec(memory_space=pl.ANY),
        out_shape=jax.ShapeDtypeStruct((B, S, D), x.dtype),
        scratch_shapes=[
            pltpu.VMEM((B, S, D), x.dtype),
            pltpu.VMEM((B + 1, S, D), x.dtype),
            pltpu.VMEM((nm + 2 * F // 128, 32, 128), f32),
            pltpu.VMEM((max(nv, 1) * (S + 1), 32, 128), f32),
            pltpu.VMEM((B + CFG["NB"], D // 128, S, 512), f32),
            pltpu.VMEM((NJ * (len(tiles[-1][0]) + 2), 32, 128), f32),
            pltpu.SemaphoreType.DMA((3,)),
            pltpu.SMEM((1,), jnp.int32),
        ],
        compiler_params=pltpu.CompilerParams(
            vmem_limit_bytes=64 * 1024 * 1024, disable_bounds_checks=True,
            flags={"XLA_TPU_FORCE_LP_LLO_SCHEDULER": True} if CFG["LP"] else None),
    )(x, w1, b1.reshape(F // 128, 128), w2.T, b2.reshape(1, S))
```

```python
import functools

import jax
import jax.experimental.pallas as pl
import jax.experimental.pallas.tpu as pltpu
import jax.numpy as jnp
import numpy as np
from jax import lax

f32, bf16, i32 = jnp.float32, jnp.bfloat16, jnp.int32

_EPS = 1e-5
_C1 = float(np.sqrt(2.0 / np.pi))
_A = float(np.cbrt(0.044715 * _C1))
_A_HI = float(np.float32(_A).astype(bf16).astype(np.float32))

_NJ = 4
_TD = 128 * _NJ
_GROUPS = 9
_UNITS = 21
_LAG = 16
_LEAD = 25
_RAW = 14
_STEP = 2
_X_TILE = 12

_Q0, _Q1, _Q2, _Q3 = (slice(128 * i, 128 * i + 128) for i in range(4))


def _mm(a, b):
    return lax.dot_general(a, b, (((1,), (0,)), ((), ())), preferred_element_type=f32)


def _pack(a):
    return pltpu.bitcast(a.astype(bf16), i32)


def _unpack(a):
    return pltpu.bitcast(a, bf16)


def _lanes(vs):
    return jnp.concatenate(list(vs), axis=1)


def _rows(vs):
    return jnp.concatenate(list(vs), axis=0)


def _act(v):
    return v * jnp.tanh(v * (v * v + _C1 / _A))


def _row_stats(x):
    mean = jnp.mean(x, axis=-1, keepdims=True)
    xc = x - mean
    return mean, lax.rsqrt(jnp.mean(xc * xc, axis=-1, keepdims=True) + _EPS) * _A


def _split_rows(n_tiles, n_units):
    vpu = [(c, r) for c in range(n_tiles) for r in (15, 14)
           if (c + 1) * n_units // n_tiles > c * n_units // n_tiles]
    mxu = [(c, r) for c in range(n_tiles) for r in range(15, -1, -1) if (c, r) not in vpu]
    return [[g[i:i + 2] for i in range(0, len(g), 2)] for g in (mxu, vpu)]


def _kernel(x_hbm, w1_hbm, b1_hbm, w2t_hbm, b2_hbm, o_hbm,
            x0_ref, x_ref, o_ref, lhs_ref, carry_ref, stat_ref, sems, zero_ref,
            w1_ref, b1_ref, w2t_ref, b2_ref, mul_ref, paced0_ref, paced1_ref, *h_refs):
    paced_refs = (paced0_ref, paced1_ref)
    B, S, D = x_hbm.shape
    n_tiles, n_half, H = w1_ref.shape[1] // 128, D // _TD, S // 2
    n_groups = B * n_half
    mxu_pairs, units = _split_rows(n_tiles, _UNITS)
    pairs = mxu_pairs + units
    i_w2 = len(pairs)
    i_lin, i_one, i_bias = (i_w2 + n_tiles + i for i in range(3))
    n_mul = 7 * H

    def mul_slot(j, k):
        if k >= n_mul or k % _STEP:
            return mul_ref, j * (n_mul + 2) + k
        step = (j * n_mul + k) // _STEP
        return paced_refs[step % 2], step // 2

    first = [pltpu.make_async_copy(src, dst, sems.at[i]) for i, (src, dst) in enumerate(
        [(x_hbm.at[0], x0_ref), (w1_hbm, w1_ref), (b1_hbm, b1_ref), (w2t_hbm, w2t_ref), (b2_hbm, b2_ref)])]
    rest = [pltpu.make_async_copy(x_hbm.at[:, :, pl.ds(z * _TD, _TD)], x_ref.at[z, pl.ds(0, B)], sems.at[6 + z])
            for z in range(n_half)]
    for cp in first:
        cp.start()
    zero_ref[0] = 0
    first[0].wait()
    x0 = x0_ref[...].astype(f32)
    mean0, scale0 = _row_stats(x0)
    x0_ref[:, :_TD] = ((x0 - mean0)[:, :_TD] * scale0).astype(bf16)
    for cp in first[1:]:
        cp.wait()
    for cp in rest:
        cp.start()
    h0 = x0_ref[:, :_TD]

    w1 = w1_ref[...].astype(f32)
    b1 = b1_ref[...].astype(f32)
    row = lax.broadcasted_iota(i32, (S, 128), 0)
    lhs_ref[i_one, :, _Q0] = _pack(jnp.where(row == 0, _A_HI, jnp.where(row == 1, _A - _A_HI, 0.0)))
    w1b = []
    for c in range(n_tiles):
        w1b.append(_rows([w1[:, 128 * c:128 * c + 128], jnp.where(row < 2, b1[c:c + 1], 0.0)]))
        wt = w1b[c].T
        lhs_ref[i_w2 + c, :, _Q0] = _pack(w2t_ref[:, 128 * c:128 * c + 128])
        for i, pair in enumerate(pairs):
            if pair[0][0] == c:
                lhs_ref[i, :, :2 * S] = _pack(_rows(wt[8 * r:8 * r + 8] for _, r in pair))
    lin = lax.dot_general(w2t_ref[...], _lanes(w1b).astype(bf16), (((1,), (1,)), ((), ())),
                          preferred_element_type=f32)
    lin_hi = lin[:, :S].astype(bf16).astype(f32)
    lhs_ref[i_lin, :, :2 * S] = _pack(_lanes([lin_hi, lin[:, :S] - lin_hi]))
    eye = lax.broadcasted_iota(i32, (S, S), 0) == lax.broadcasted_iota(i32, (S, S), 1)
    b2 = jnp.sum(jnp.where(eye, b2_ref[...].astype(f32), 0.0), axis=1, keepdims=True)
    bias = jnp.broadcast_to(b2 + 0.5 * lin[:, S:S + 1], (S, 128))
    for z in range(2):
        lhs_ref[i_bias + z, :, _Q0] = pltpu.bitcast(bias[8 * z:8 * z + 8], i32)

    def prepare_unit(j):
        w = _unpack(lhs_ref[len(mxu_pairs) + j, :, :2 * S]).astype(f32)
        col = lambda g, k: jnp.broadcast_to(w[8 * g:8 * g + 8, k:k + 1], (8, 128))
        for k in range(H):
            a11, a12, a21, a22 = col(0, k), col(0, H + k), col(1, k), col(1, H + k)
            s1 = a21 + a22
            s2 = s1 - a11
            for z, v in enumerate([a11, a12, s2, s1, a12 - s2, a11 - a21, a22]):
                ref, i = mul_slot(j, z * H + k)
                ref[i, :, _Q1] = v
        for k, v in enumerate([col(0, S), col(1, S) - col(0, S)]):
            ref, i = mul_slot(j, n_mul + k)
            ref[i, :, _Q1] = v * _A

    def normalize(q, cg):
        b = cg // n_half
        mean, scale = (jnp.tile(stat_ref[b, :, s], (1, _NJ)) for s in (_Q0, _Q1))
        h = (x_ref[cg % n_half, b].astype(f32) - mean) * scale
        for p in range(_NJ // 2):
            b11, b12 = h[:H, 256 * p:256 * p + 128], h[:H, 256 * p + 128:256 * p + 256]
            b21, b22 = h[H:, 256 * p:256 * p + 128], h[H:, 256 * p + 128:256 * p + 256]
            t1 = b12 - b11
            t2 = b22 - t1
            for z, v in enumerate([b11, b21, t2, t1, b22, b22 - b12, b21 - t2]):
                h_refs[q][7 * p + z, :, _Q2] = v
        return h.astype(bf16)

    def vpu_unit(q, j, h_row, acts):
        load = lambda ref, i: ref[i, :, _Q1]
        add = lambda xs, ys: [x + y for x, y in zip(xs, ys)]

        def product(z, accs=None):
            for k in range(H):
                if (z * H + k) % _STEP == 0:
                    yield mul_slot(j, z * H + k)[0]
                w = load(*mul_slot(j, z * H + k))
                terms = [w * h_row(q, 7 * p + z, k) for p in range(_NJ // 2)]
                accs = add(accs, terms) if accs else terms
            return accs

        p1 = yield from product(0, [load(*mul_slot(j, n_mul))] * 2)
        c11 = [_act(v) for v in add(p1, (yield from product(1)))]
        u2 = add(p1, (yield from product(2)))
        p5 = yield from product(3)
        c12 = [_act(v) for v in add(add(u2, p5), (yield from product(4)))]
        acts[(q,) + units[j][0]] = _lanes([c11[0], c12[0], c11[1], c12[1]])
        u3 = add(u2, (yield from product(5, [load(*mul_slot(j, n_mul + 1))] * 2)))
        c22 = [_act(v) for v in add(u3, p5)]
        c21 = [_act(v) for v in add(u3, (yield from product(6)))]
        acts[(q,) + units[j][1]] = _lanes([c21[0], c22[0], c21[1], c22[1]])

    def second_matmul(c, g):
        return _mm(_unpack(lhs_ref[i_w2 + c, :, _Q0]), _rows(g))

    def linear_half(h):
        return _mm(_unpack(lhs_ref[i_lin, :, :2 * S]), _rows([h, h]))

    def carry_load(r):
        return _lanes(carry_ref[_NJ * r + jj, :, _Q3] for jj in range(_NJ))

    def carry_store(r, v):
        for jj in range(_NJ):
            carry_ref[_NJ * r + jj, :, _Q3] = v[:, 128 * jj:128 * jj + 128]

    def emit(cg, acc):
        bias = _rows(pltpu.bitcast(lhs_ref[i_bias + z, :, _Q0], f32) for z in range(2))
        o_ref[cg] = (acc * (0.5 / _A) + jnp.tile(bias, (1, _NJ))).astype(o_ref.dtype)
        cols = pl.ds(pl.multiple_of(cg % n_half * _TD, _TD), _TD)
        pltpu.make_async_copy(o_ref.at[cg], o_hbm.at[cg // n_half, :, cols], sems.at[5]).start()

    def finish_carried(cg):
        g = [carry_load(r) for r in range(18)]
        emit(cg, _rows(g[16:]) + second_matmul(n_tiles - 1, [_act(g[r]) if r < _RAW else g[r] for r in range(16)]))

    def block(cg0, n_cg, todo, hs, after_tile):
        warm_up = not todo
        flat, ends = [], [(-1, n_tiles - 1, 0)]
        for q in range(n_cg):
            idx = [i for i in range(len(pairs)) if (q, i - len(mxu_pairs)) not in todo]
            idx.sort(key=lambda i: (pairs[i][0][0], -pairs[i][0][1]))
            ends += [(q, c, 2 * (len(flat) + sum(pairs[i][0][0] <= c for i in idx))) for c in range(n_tiles)]
            flat += [(q, i) for i in idx]
        ends.pop()
        acts, acc = {}, {}

        @functools.cache
        def h_row(q, i, k):
            return jnp.broadcast_to(h_refs[q][i, k:k + 1, _Q2], (8, 128))

        def vpu_stream():
            for q, j in todo:
                yield from vpu_unit(q, j, h_row, acts)

        clock = np.arange(2 * len(flat)) - 2.0
        for _, _, n in ends:
            clock[n + _LAG:] += 2
        span = 2 * (len(mxu_pairs) + n_tiles) / len(units)
        when = [int(np.searchsorted(clock, (q * len(units) + j + k / n_mul) * span - _LEAD + 1e-6)) - 1
                for q, j in todo for k in range(0, n_mul, _STEP)]
        stream = vpu_stream()
        state = [0, next(stream, None)]
        zero = zero_ref[0]

        def pace(t, u):
            while state[0] < len(when) and when[state[0]] <= t:
                if u is not None:
                    state[1][zero, :, _Q3] = u[:, -128:]
                state[:] = state[0] + 1, next(stream, None)

        pace(-1, None)
        pos = 0
        for q, c, n in ends:
            target = min((n + _LAG) // 2, len(flat))
            us = []
            while pos < target:
                q1 = flat[pos][0]
                stop = max(t + 1 for t in range(pos, target) if flat[t][0] == q1)
                if not warm_up and (pos == 0 or flat[pos - 1][0] != q1):
                    acc[q1] = linear_half(hs[q1])
                rhs = _rows([hs[q1], jnp.tile(_unpack(lhs_ref[i_one, :, _Q0]), (1, _NJ))])
                u = _mm(_rows(_unpack(lhs_ref[i, :, :2 * S]) for _, i in flat[pos:stop]), rhs)
                for t in range(2 * pos, 2 * stop):
                    v = u[8 * (t - 2 * pos):8 * (t - 2 * pos) + 8]
                    c1, r = pairs[flat[t // 2][1]][t % 2]
                    acts[q1, c1, r] = v if (q1, c1) == (n_cg - 1, n_tiles - 1) and r < _RAW else _act(v)
                    us.append((t, v))
                pos = stop
            for t, v in us:
                pace(t, v)
            if q < 0:
                if not warm_up:
                    finish_carried(cg0 - 1)
                continue
            if warm_up and c == n_tiles - 4:
                acc[q] += linear_half(hs[q])
            part = second_matmul(c, [acts.pop((q, c, r)) for r in range(16)])
            if c > 0 and not warm_up:
                acc[q] = _rows([carry_load(16), carry_load(17)])
            acc[q] = acc[q] + part if q in acc else part
            if c == n_tiles - 1:
                emit(cg0 + q, acc.pop(q))
            elif not warm_up or c == n_tiles - 2:
                carry_store(16, acc[q][:8])
                carry_store(17, acc[q][8:])
            after_tile(q, c, us)
        assert state[1] is None
        for r in range(16):
            carry_store(r, acts.pop((n_cg - 1, n_tiles - 1, r)))

    def prepare(q, c, us):
        for j in range(len(units)):
            if 1 + j * (_X_TILE - 1) // len(units) == c:
                prepare_unit(j)
        if c == _X_TILE:
            for cp in rest:
                cp.wait()
        for b in range(B + 1):
            t = (_X_TILE + 1) * 16 + b * (n_tiles - 4 - _X_TILE) * 16 // B
            if t // 16 == c:
                x_ref[0, B + zero_ref[0], :, _Q0] = _rows([us[t % 16][1][:, _Q0]] * 2).astype(bf16)
                if b < B:
                    mean, scale = _row_stats(_lanes(x_ref[z, b].astype(f32) for z in range(n_half)))
                    stat_ref[b, :, _Q0] = jnp.broadcast_to(mean, (S, 128))
                    stat_ref[b, :, _Q1] = jnp.broadcast_to(scale, (S, 128))

    block(0, 1, [], [h0], prepare)

    @pl.loop(0, (n_groups - 1) // len(h_refs))
    def _(it):
        cg0 = 1 + it * len(h_refs)
        hs = [normalize(0, cg0)]

        def next_group(q, c, us):
            if c == n_tiles - 8 and q + 1 < len(h_refs):
                hs.append(normalize(q + 1, cg0 + q + 1))

        todo = [(q, j) for q in range(len(h_refs)) for j in range(len(units))][1:-1]
        block(cg0, len(h_refs), todo, hs, next_group)

    finish_carried(n_groups - 1)
    pltpu.make_async_copy(o_hbm, o_hbm, sems.at[5]).wait()


@jax.jit
def pallas_standalone__mixer_token_mlp__sampling_kernel(
    x: jax.Array,
    w1: jax.Array,
    b1: jax.Array,
    w2: jax.Array,
    b2: jax.Array,
):
    B, S, D = x.shape
    F = w1.shape[1]
    assert S == 16 and D % _TD == 0 and F % 128 == 0 and (B * D // _TD - 1) % _GROUPS == 0
    small = (w1, b1.reshape(F // 128, 128), w2.T, b2.reshape(1, S))
    slab = lambda n, dtype: pltpu.VMEM((n, 8, 512), dtype)
    n_mul = 7 * S // 2
    return pl.pallas_call(
        _kernel,
        in_specs=[pl.BlockSpec(memory_space=pl.ANY)] * 5,
        out_specs=pl.BlockSpec(memory_space=pl.ANY),
        out_shape=jax.ShapeDtypeStruct((B, S, D), x.dtype),
        scratch_shapes=[
            pltpu.VMEM((S, D), x.dtype),
            pltpu.VMEM((D // _TD, B + 1, S, _TD), x.dtype),
            pltpu.VMEM((B * D // _TD, S, _TD), x.dtype),
            slab(F // 16 + F // 128 + 4, i32),
            slab(_NJ * 18, f32),
            pltpu.VMEM((B, S, 256), f32),
            pltpu.SemaphoreType.DMA((6 + D // _TD,)),
            pltpu.SMEM((1,), i32),
            *[pltpu.VMEM(a.shape, a.dtype) for a in small],
            slab(_UNITS * (n_mul + 2), f32),
            *[slab(_UNITS * n_mul // _STEP // 2, f32)] * 2,
            *[slab(7 * _NJ // 2, f32)] * _GROUPS,
        ],
        compiler_params=pltpu.CompilerParams(vmem_limit_bytes=128 * 1024 * 1024),
    )(x, *small)
```

```python
import functools

import jax
import jax.experimental.pallas as pl
import jax.experimental.pallas.tpu as pltpu
import jax.numpy as jnp
import numpy as np
from jax import lax

f32, bf16, i32 = jnp.float32, jnp.bfloat16, jnp.int32

_EPS = 1e-5
_C1 = float(np.sqrt(2.0 / np.pi))
_A = float(np.cbrt(0.044715 * _C1))
_A_HI = float(np.float32(_A).astype(bf16).astype(np.float32))

_NJ = 4
_TD = 128 * _NJ
_GROUPS = 9
_UNITS = 21
_LAG = 16
_LEAD = 25
_STEP = 2
_HEAD = 3
_X_TILE = 13

_Q0, _Q1, _Q2, _Q3 = (slice(128 * i, 128 * i + 128) for i in range(4))


def _mm(a, b):
    return lax.dot_general(a, b, (((1,), (0,)), ((), ())), preferred_element_type=f32)


def _pack(a):
    return pltpu.bitcast(a.astype(bf16), i32)


def _unpack(a):
    return pltpu.bitcast(a, bf16)


def _lanes(vs):
    return jnp.concatenate(list(vs), axis=1)


def _rows(vs):
    return jnp.concatenate(list(vs), axis=0)


def _act(v):
    return v * jnp.tanh(v * (v * v + _C1 / _A))


def _row_stats(x):
    mean = jnp.mean(x, axis=-1, keepdims=True)
    xc = x - mean
    return mean, lax.rsqrt(jnp.mean(xc * xc, axis=-1, keepdims=True) + _EPS) * _A


def _split_rows(n_tiles, n_units):
    vpu, n = [], 8 * n_tiles
    for i in range(n):
        if (i + 1) * n_units // n > i * n_units // n:
            c, p = i // 8, 2 * (i % 8)
            vpu += [(c, 15 - max(p - 9, 0)), (c, 15 - max(p - 6, 1))]
    mxu = [(c, r) for c in range(n_tiles) for r in range(15, -1, -1) if (c, r) not in vpu]
    return [[g[i:i + 2] for i in range(0, len(g), 2)] for g in (mxu, vpu)]


def _kernel(x_hbm, w1_hbm, b1_hbm, w2t_hbm, b2_hbm, o_hbm,
            x0_ref, x_ref, o_ref, lhs_ref, carry_ref, stat_ref, sems, zero_ref,
            w1_head_ref, w1_tail_ref, b1_ref, w2t_ref, b2_ref, mul_ref, paced0_ref, paced1_ref, *h_refs):
    paced_refs = (paced0_ref, paced1_ref)
    B, S, D = x_hbm.shape
    n_tiles, n_half, H = w1_hbm.shape[1] // 128, D // _TD, S // 2
    n_groups = B * n_half
    mxu_pairs, units = _split_rows(n_tiles, _UNITS)
    pairs = mxu_pairs + units
    i_w2 = len(pairs)
    i_lin, i_one, i_bias = (i_w2 + n_tiles + i for i in range(3))
    n_mul = 7 * H

    def mul_slot(j, k):
        if k >= n_mul or (k + 1) % _STEP:
            return mul_ref, j * (n_mul + 2) + k
        step = (j * n_mul + k) // _STEP
        return paced_refs[step % 2], step // 2

    head, tail = pl.ds(0, 128 * _HEAD), pl.ds(128 * _HEAD, 128 * (n_tiles - _HEAD))
    loads = [pltpu.make_async_copy(src, dst, sems.at[1 + i]) for i, (src, dst) in enumerate(
        [(x_hbm.at[0], x0_ref), (w1_hbm.at[:, head], w1_head_ref), (b1_hbm, b1_ref),
         (w1_hbm.at[:, tail], w1_tail_ref), (w2t_hbm, w2t_ref), (b2_hbm, b2_ref)]
        + [(x_hbm.at[:, :, pl.ds(z * _TD, _TD)], x_ref.at[z, pl.ds(0, B)]) for z in range(n_half)])]
    for cp in loads[:6]:
        cp.start()
    zero_ref[0] = 0
    row = lax.broadcasted_iota(i32, (S, 128), 0)
    lhs_ref[i_one, :, _Q0] = _pack(jnp.where(row == 0, _A_HI, jnp.where(row == 1, _A - _A_HI, 0.0)))

    def w1_and_bias(c):
        b1 = b1_ref[...].astype(f32)[c:c + 1]
        ref, i = (w1_head_ref, c) if c < _HEAD else (w1_tail_ref, c - _HEAD)
        return _rows([ref[:, 128 * i:128 * i + 128].astype(f32), jnp.where(row < 2, b1, 0.0)])

    def prepare_tile(c):
        wt = w1_and_bias(c).T
        for i, pair in enumerate(pairs):
            if pair[0][0] == c:
                lhs_ref[i, :, :2 * S] = _pack(_rows(wt[8 * r:8 * r + 8] for _, r in pair))

    for cp in loads[:3]:
        cp.wait()
    x0 = x0_ref[...].astype(f32)
    mean0, scale0 = _row_stats(x0)
    x0_ref[:, :_TD] = ((x0 - mean0)[:, :_TD] * scale0).astype(bf16)
    for c in range(_HEAD):
        prepare_tile(c)
    for cp in loads[3:6]:
        cp.wait()
    for cp in loads[6:]:
        cp.start()
    h0 = x0_ref[:, :_TD]
    for c in range(n_tiles):
        lhs_ref[i_w2 + c, :, _Q0] = _pack(w2t_ref[:, 128 * c:128 * c + 128])
        if c >= _HEAD:
            prepare_tile(c)

    def prepare_linear():
        w1b = _lanes(w1_and_bias(c) for c in range(n_tiles)).astype(bf16)
        lin = lax.dot_general(w2t_ref[...], w1b, (((1,), (1,)), ((), ())), preferred_element_type=f32)
        lin_hi = lin[:, :S].astype(bf16).astype(f32)
        lhs_ref[i_lin, :, :2 * S] = _pack(_lanes([lin_hi, lin[:, :S] - lin_hi]))
        eye = lax.broadcasted_iota(i32, (S, S), 0) == lax.broadcasted_iota(i32, (S, S), 1)
        b2 = jnp.sum(jnp.where(eye, b2_ref[...].astype(f32), 0.0), axis=1, keepdims=True)
        bias = jnp.broadcast_to(b2 + 0.5 * lin[:, S:S + 1], (S, 128))
        for z in range(2):
            lhs_ref[i_bias + z, :, _Q0] = pltpu.bitcast(bias[8 * z:8 * z + 8], i32)

    def prepare_unit(j):
        w = _unpack(lhs_ref[len(mxu_pairs) + j, :, :2 * S]).astype(f32)
        col = lambda g, k: jnp.broadcast_to(w[8 * g:8 * g + 8, k:k + 1], (8, 128))
        for k in range(H):
            a11, a12, a21, a22 = col(0, k), col(0, H + k), col(1, k), col(1, H + k)
            s1 = a21 + a22
            s2 = s1 - a11
            for z, v in enumerate([a11, a12, s2, s1, a12 - s2, a11 - a21, a22]):
                ref, i = mul_slot(j, z * H + k)
                ref[i, :, _Q1] = v
        for k, v in enumerate([col(0, S), col(1, S) - col(0, S)]):
            ref, i = mul_slot(j, n_mul + k)
            ref[i, :, _Q1] = v * _A

    def normalize(q, cg):
        b = cg // n_half
        mean, scale = (jnp.tile(stat_ref[b, :, s], (1, _NJ)) for s in (_Q0, _Q1))
        h = (x_ref[cg % n_half, b].astype(f32) - mean) * scale
        for p in range(_NJ // 2):
            b11, b12 = h[:H, 256 * p:256 * p + 128], h[:H, 256 * p + 128:256 * p + 256]
            b21, b22 = h[H:, 256 * p:256 * p + 128], h[H:, 256 * p + 128:256 * p + 256]
            t1 = b12 - b11
            t2 = b22 - t1
            for z, v in enumerate([b11, b21, t2, t1, b22, b22 - b12, b21 - t2]):
                h_refs[q][7 * p + z, :, _Q2] = v
        return h.astype(bf16)

    def vpu_unit(q, j, h_row, acts):
        load = lambda ref, i: ref[i, :, _Q1]
        add = lambda xs, ys: [x + y for x, y in zip(xs, ys)]

        def product(z, accs=None):
            for k in range(H):
                if (z * H + k) % _STEP == 0:
                    yield mul_slot(j, z * H + k + _STEP - 1)[0]
                w = load(*mul_slot(j, z * H + k))
                terms = [w * h_row(q, 7 * p + z, k) for p in range(_NJ // 2)]
                accs = add(accs, terms) if accs else terms
            return accs

        p1 = yield from product(0, [load(*mul_slot(j, n_mul))] * 2)
        c11 = [_act(v) for v in add(p1, (yield from product(1)))]
        u2 = add(p1, (yield from product(2)))
        p5 = yield from product(3)
        c12 = [_act(v) for v in add(add(u2, p5), (yield from product(4)))]
        acts[(q,) + units[j][0]] = _lanes([c11[0], c12[0], c11[1], c12[1]])
        u3 = add(u2, (yield from product(5, [load(*mul_slot(j, n_mul + 1))] * 2)))
        c22 = [_act(v) for v in add(u3, p5)]
        c21 = [_act(v) for v in add(u3, (yield from product(6)))]
        acts[(q,) + units[j][1]] = _lanes([c21[0], c22[0], c21[1], c22[1]])

    def second_matmul(c, g):
        return _mm(_unpack(lhs_ref[i_w2 + c, :, _Q0]), _rows(g))

    def linear_half(h):
        return _mm(_unpack(lhs_ref[i_lin, :, :2 * S]), _rows([h, h]))

    def carry_load(r):
        return _lanes(carry_ref[_NJ * r + jj, :, _Q3] for jj in range(_NJ))

    def carry_store(r, v):
        for jj in range(_NJ):
            carry_ref[_NJ * r + jj, :, _Q3] = v[:, 128 * jj:128 * jj + 128]

    def emit(cg, acc):
        bias = _rows(pltpu.bitcast(lhs_ref[i_bias + z, :, _Q0], f32) for z in range(2))
        o_ref[cg] = (acc * (0.5 / _A) + jnp.tile(bias, (1, _NJ))).astype(o_ref.dtype)
        cols = pl.ds(pl.multiple_of(cg % n_half * _TD, _TD), _TD)
        pltpu.make_async_copy(o_ref.at[cg], o_hbm.at[cg // n_half, :, cols], sems.at[0]).start()

    def finish_carried(cg):
        g = [carry_load(r) for r in range(18)]
        emit(cg, _rows(g[16:]) + second_matmul(n_tiles - 1, g[:16]))

    def block(cg0, n_cg, todo, hs, after_tile):
        warm_up = not todo
        flat, ends = [], [(-1, n_tiles - 1, 0)]
        for q in range(n_cg):
            idx = [i for i in range(len(pairs)) if (q, i - len(mxu_pairs)) not in todo]
            idx.sort(key=lambda i: (pairs[i][0][0], -pairs[i][0][1]))
            ends += [(q, c, 2 * (len(flat) + sum(pairs[i][0][0] <= c for i in idx))) for c in range(n_tiles)]
            flat += [(q, i) for i in idx]
        ends.pop()
        acts, acc = {}, {}

        @functools.cache
        def h_row(q, i, k):
            return jnp.broadcast_to(h_refs[q][i, k:k + 1, _Q2], (8, 128))

        def vpu_stream():
            for q, j in todo:
                yield from vpu_unit(q, j, h_row, acts)

        clock = np.arange(2 * len(flat)) - 2.0
        for _, _, n in ends:
            clock[n + _LAG:] += 1.5
        span = (2 * len(mxu_pairs) + 1.5 * n_tiles) / len(units)
        when = [int(np.searchsorted(clock, (q * len(units) + j + k / n_mul) * span - _LEAD + 1e-6)) - 1
                for q, j in todo for k in range(0, n_mul, _STEP)]
        stream = vpu_stream()
        state = [0, next(stream, None)]
        zero = zero_ref[0]

        def pace(t, u):
            while state[0] < len(when) and when[state[0]] <= t:
                if u is not None:
                    state[1][zero, :, _Q3] = u[:, _Q2]
                state[:] = state[0] + 1, next(stream, None)

        pace(-1, None)
        pos = 0
        for q, c, n in ends:
            target = min((n + _LAG) // 2, len(flat))
            us = []
            while pos < target:
                q1 = flat[pos][0]
                stop = max(t + 1 for t in range(pos, target) if flat[t][0] == q1)
                if not warm_up and (pos == 0 or flat[pos - 1][0] != q1):
                    acc[q1] = linear_half(hs[q1])
                rhs = _rows([hs[q1], jnp.tile(_unpack(lhs_ref[i_one, :, _Q0]), (1, _NJ))])
                u = _mm(_rows(_unpack(lhs_ref[i, :, :2 * S]) for _, i in flat[pos:stop]), rhs)
                for t in range(2 * pos, 2 * stop):
                    v = u[8 * (t - 2 * pos):8 * (t - 2 * pos) + 8]
                    acts[(q1,) + pairs[flat[t // 2][1]][t % 2]] = _act(v)
                    us.append((t, v))
                pos = stop
            for t, v in us:
                pace(t, v)
            if q < 0:
                if warm_up:
                    prepare_linear()
                else:
                    finish_carried(cg0 - 1)
                continue
            if warm_up and c == n_tiles - 4:
                acc[q] += linear_half(hs[q])
            part = second_matmul(c, [acts.pop((q, c, r)) for r in range(16)])
            acc[q] = acc[q] + part if q in acc else part
            if c == n_tiles - 1:
                emit(cg0 + q, acc.pop(q))
            elif (q, c) == (n_cg - 1, n_tiles - 2):
                carry_store(16, acc[q][:8])
                carry_store(17, acc[q][8:])
            after_tile(q, c, us)
        assert state[1] is None
        for r in range(16):
            carry_store(r, acts.pop((n_cg - 1, n_tiles - 1, r)))

    def prepare(q, c, us):
        for j in range(len(units)):
            if 1 + j * (_X_TILE - 1) // len(units) == c:
                prepare_unit(j)
        if c == _X_TILE:
            for cp in loads[6:]:
                cp.wait()
        for b in range(B + 1):
            t = (_X_TILE + 1) * 16 + b * (n_tiles - 4 - _X_TILE) * 16 // B
            if t // 16 == c:
                x_ref[0, B + zero_ref[0], :, _Q0] = _rows([us[t % 16][1][:, _Q0]] * 2).astype(bf16)
                if b < B:
                    mean, scale = _row_stats(_lanes(x_ref[z, b].astype(f32) for z in range(n_half)))
                    stat_ref[b, :, _Q0] = jnp.broadcast_to(mean, (S, 128))
                    stat_ref[b, :, _Q1] = jnp.broadcast_to(scale, (S, 128))

    block(0, 1, [], [h0], prepare)

    @pl.loop(0, (n_groups - 1) // len(h_refs))
    def _(it):
        cg0 = 1 + it * len(h_refs)
        hs = [normalize(0, cg0)]

        def next_group(q, c, us):
            if c == n_tiles - 8 and q + 1 < len(h_refs):
                hs.append(normalize(q + 1, cg0 + q + 1))

        todo = [(q, j) for q in range(len(h_refs)) for j in range(len(units))][1:-1]
        block(cg0, len(h_refs), todo, hs, next_group)

    finish_carried(n_groups - 1)
    pltpu.make_async_copy(o_hbm, o_hbm, sems.at[0]).wait()


@jax.jit
def pallas_standalone__mixer_token_mlp__sampling_kernel(
    x: jax.Array,
    w1: jax.Array,
    b1: jax.Array,
    w2: jax.Array,
    b2: jax.Array,
):
    B, S, D = x.shape
    F = w1.shape[1]
    assert S == 16 and D % _TD == 0 and F % 128 == 0 and (B * D // _TD - 1) % _GROUPS == 0
    small = (b1.reshape(F // 128, 128), w2.T, b2.reshape(1, S))
    slab = lambda n, dtype: pltpu.VMEM((n, 8, 512), dtype)
    n_mul = 7 * S // 2
    return pl.pallas_call(
        _kernel,
        in_specs=[pl.BlockSpec(memory_space=pl.ANY)] * 5,
        out_specs=pl.BlockSpec(memory_space=pl.ANY),
        out_shape=jax.ShapeDtypeStruct((B, S, D), x.dtype),
        scratch_shapes=[
            pltpu.VMEM((S, D), x.dtype),
            pltpu.VMEM((D // _TD, B + 1, S, _TD), x.dtype),
            pltpu.VMEM((B * D // _TD, S, _TD), x.dtype),
            slab(F // 16 + F // 128 + 4, i32),
            slab(_NJ * 18, f32),
            pltpu.VMEM((B, S, 256), f32),
            pltpu.SemaphoreType.DMA((7 + D // _TD,)),
            pltpu.SMEM((1,), i32),
            pltpu.VMEM((S, 128 * _HEAD), w1.dtype),
            pltpu.VMEM((S, F - 128 * _HEAD), w1.dtype),
            *[pltpu.VMEM(a.shape, a.dtype) for a in small],
            slab(_UNITS * (n_mul + 2), f32),
            *[slab(_UNITS * n_mul // _STEP // 2, f32)] * 2,
            *[slab(7 * _NJ // 2, f32)] * _GROUPS,
        ],
        compiler_params=pltpu.CompilerParams(vmem_limit_bytes=128 * 1024 * 1024),
    )(x, w1, *small)
```
